```python
import os as _os
_os.environ.setdefault("JAX_PLATFORMS", "cpu")
import jax
import jax.numpy as jnp

def _softmax(x, axis=-1):
    return jax.nn.softmax(x, axis=axis)
def _gelu(x):
    return jax.nn.gelu(x, approximate=True)
def _silu(x):
    return jax.nn.silu(x)
def _sigmoid(x):
    return jax.nn.sigmoid(x)
def _layernorm(x, axis=-1, eps=1e-5):
    m = jnp.mean(x, axis=axis, keepdims=True)
    v = jnp.var(x, axis=axis, keepdims=True)
    return (x - m) / jnp.sqrt(v + eps)
def _scatter_add(tgt, idx, src, axis=0):
    return tgt.at[idx].add(src)
def _segment_sum(src, seg, n):
    return jax.ops.segment_sum(src, seg, n)
class _Rng:
    def __init__(self, key):
        self._k = key
    def _next(self):
        self._k, sub = jax.random.split(self._k)
        return sub
    def normal(self, shape):
        return jax.random.normal(self._next(), shape, dtype=jnp.bfloat16)
    def randint(self, lo, hi, shape):
        return jax.random.randint(self._next(), shape, lo, hi, dtype=jnp.int32)
    def uniform(self, shape, lo=0.0, hi=1.0):
        return jax.random.uniform(self._next(), shape, jnp.bfloat16, lo, hi)
    def permutation(self, n):
        return jax.random.permutation(self._next(), n)


kernel_name = 'parallel_sum__sliding_local_dilated__glu_gated_geglu__prompt'

def setup_inputs():
    _rng = _Rng(jax.random.key(int.from_bytes(__import__("os").urandom(4), "little")))
    _w = (lambda a: (lambda t: t.astype(jnp.bfloat16) if jnp.issubdtype(t.dtype, jnp.floating) else t)(jnp.asarray(a)))
    def _A_setup():
        B, S, D = 1, 2048, 512
        return {
            "x": _w((lambda *s: _rng.normal(s) * 0.05)(B, S, D)),
            "wqkv": _w((lambda *s: _rng.normal(s) * 0.05)(D, 3 * D)),
            "wo": _w((lambda *s: _rng.normal(s) * 0.05)(D, D)),
        }
    _A_in = _A_setup()

    def _B_setup():
        B, S, Dm, Df = 1, 2048, 512, 1376
        return {
            "x": _w((lambda *s: _rng.normal(s) * 0.05)(B, S, Dm)),
            "w_gate": _w((lambda *s: _rng.normal(s) * 0.1)(Dm, Df) * (Dm ** -0.5)),
            "w_up": _w((lambda *s: _rng.normal(s) * 0.1)(Dm, Df) * (Dm ** -0.5)),
            "w_down": _w((lambda *s: _rng.normal(s) * 0.1)(Df, Dm) * (Df ** -0.5)),
        }
    _B_in = _B_setup()

    return {
        "A_x": _A_in["x"],
        "A_wqkv": _A_in["wqkv"],
        "A_wo": _A_in["wo"],
        "B_x": _B_in["x"],
        "B_w_gate": _B_in["w_gate"],
        "B_w_up": _B_in["w_up"],
        "B_w_down": _B_in["w_down"],
    }

def reference(A_x, A_wqkv, A_wo, B_x, B_w_gate, B_w_up, B_w_down):
    def _A_ref(x, wqkv, wo):
        B, S, D = x.shape
        H = 32; Dh = D // H
        W, dil = 8, 2
        qkv = (lambda x, *d: x.transpose(*d))((x @ wqkv).reshape(B, S, 3, H, Dh), 2, 0, 3, 1, 4)
        q, k, v = qkv[0], qkv[1], qkv[2]
        scale = Dh ** -0.5
        pos = jnp.arange(S)
        off = jnp.arange(W) * dil
        idx = pos[:, None] - off[None, :]
        mask = idx >= 0
        idx_c = jnp.where(mask, idx, 0).reshape(-1)
        kg = k[:, :, idx_c, :].reshape(B, H, S, W, Dh)
        vg = v[:, :, idx_c, :].reshape(B, H, S, W, Dh)
        logits = jnp.einsum("bhsd,bhswd->bhsw", q, kg) * scale
        logits = jnp.where(mask[None, None, :, :], logits, -1e9)
        attn = _softmax(logits, axis=-1)
        o = jnp.einsum("bhsw,bhswd->bhsd", attn, vg)
        return (lambda x, *d: x.transpose(*d))(o, 0, 2, 1, 3).reshape(B, S, D) @ wo

    def _B_ref(x, w_gate, w_up, w_down):
        g = jnp.einsum("bsd,df->bsf", x, w_gate)
        u = jnp.einsum("bsd,df->bsf", x, w_up)
        h = _gelu(g) * u
        return jnp.einsum("bsf,fd->bsd", h, w_down)

    x = A_x
    xn = _layernorm(x, axis=-1)
    return x + _A_ref(xn, A_wqkv, A_wo) + _B_ref(xn, B_w_gate, B_w_up, B_w_down)
```

```python
import functools

import jax
import jax.numpy as jnp
import jax.experimental.pallas as pl
import jax.experimental.pallas.tpu as pltpu

H = 32
DH = 16
WIN = 8
DIL = 2
HALO = 16
LANES = 128
EPS = 1e-5
NEG = -1e9


def _gelu_tanh(x):
    c = 0.7978845608028654
    return 0.5 * x * (1.0 + jnp.tanh(c * (x + 0.044715 * (x * x * x))))


def _kernel(x_ref, wqkv_hbm, wo_hbm, wg_hbm, wu_hbm, wd_hbm, out_ref,
            wqkv_raw, wo_raw, wqkv_p, wo_p, wg, wu, wd,
            qbuf, kbuf, vbuf, obuf, sems, *, T, R, D):
    i = pl.program_id(0)
    NC = D // LANES

    @pl.when(i == 0)
    def _():
        cp_wo = pltpu.make_async_copy(wo_hbm, wo_raw, sems.at[0])
        cp_qkv = pltpu.make_async_copy(wqkv_hbm, wqkv_raw, sems.at[1])
        cp_g = pltpu.make_async_copy(wg_hbm, wg, sems.at[2])
        cp_u = pltpu.make_async_copy(wu_hbm, wu, sems.at[3])
        cp_d = pltpu.make_async_copy(wd_hbm, wd, sems.at[4])
        cp_wo.start()
        cp_qkv.start()
        cp_g.start()
        cp_u.start()
        cp_d.start()

        kbuf[:, T:T + HALO, :] = jnp.zeros((NC, HALO, LANES), jnp.float32)
        vbuf[:, T:T + HALO, :] = jnp.zeros((NC, HALO, LANES), jnp.float32)

        r = jax.lax.broadcasted_iota(jnp.int32, (D, D), 0)
        c = jax.lax.broadcasted_iota(jnp.int32, (D, D), 1)
        p_old_new = (r == (c % H) * DH + c // H)
        p_new_old = (c == (r % H) * DH + r // H)
        pm = jnp.where(p_old_new, 1.0, 0.0).astype(jnp.bfloat16)
        pmq = jnp.where(p_old_new, DH ** -0.5, 0.0).astype(jnp.bfloat16)
        pmt = jnp.where(p_new_old, 1.0, 0.0).astype(jnp.bfloat16)

        cp_wo.wait()
        wo_p[...] = jnp.dot(pmt, wo_raw[...],
                            preferred_element_type=jnp.float32).astype(jnp.bfloat16)
        cp_qkv.wait()
        wqkv_p[:, 0:D] = jnp.dot(wqkv_raw[:, 0:D], pmq,
                                 preferred_element_type=jnp.float32).astype(jnp.bfloat16)
        wqkv_p[:, D:2 * D] = jnp.dot(wqkv_raw[:, D:2 * D], pm,
                                     preferred_element_type=jnp.float32).astype(jnp.bfloat16)
        wqkv_p[:, 2 * D:3 * D] = jnp.dot(wqkv_raw[:, 2 * D:3 * D], pm,
                                         preferred_element_type=jnp.float32).astype(jnp.bfloat16)
        cp_g.wait()
        cp_u.wait()
        cp_d.wait()

    kbuf[:, 0:HALO, :] = kbuf[:, T:T + HALO, :]
    vbuf[:, 0:HALO, :] = vbuf[:, T:T + HALO, :]

    x = x_ref[...].astype(jnp.float32)
    mu = jnp.mean(x, axis=-1, keepdims=True)
    xc = x - mu
    var = jnp.mean(xc * xc, axis=-1, keepdims=True)
    xn = (xc * jax.lax.rsqrt(var + EPS)).astype(jnp.bfloat16)

    qkv = jnp.dot(xn, wqkv_p[...], preferred_element_type=jnp.float32)
    for c in range(NC):
        qbuf[c] = qkv[:, c * LANES:(c + 1) * LANES]
        kbuf[c, HALO:HALO + T, :] = qkv[:, D + c * LANES:D + (c + 1) * LANES]
        vbuf[c, HALO:HALO + T, :] = qkv[:, 2 * D + c * LANES:2 * D + (c + 1) * LANES]

    for r0 in range(0, T, R):
        qc = [qbuf[c, r0:r0 + R, :] for c in range(NC)]
        ls = []
        for w in range(WIN):
            s0 = HALO + r0 - DIL * w
            p = qc[0] * kbuf[0, s0:s0 + R, :]
            for c in range(1, NC):
                p = p + qc[c] * kbuf[c, s0:s0 + R, :]
            p = p + pltpu.roll(p, 64, 1)
            p = p + pltpu.roll(p, 32, 1)
            if r0 < HALO and w > 0:
                pos = i * T + r0 + jax.lax.broadcasted_iota(jnp.int32, (R, LANES), 0)
                p = jnp.where(pos >= DIL * w, p, NEG)
            ls.append(p)
        m = ls[0]
        for w in range(1, WIN):
            m = jnp.maximum(m, ls[w])
        es = [jnp.exp(l - m) for l in ls]
        den = es[0]
        for w in range(1, WIN):
            den = den + es[w]
        inv = 1.0 / den
        for c in range(NC):
            acc = es[0] * vbuf[c, HALO + r0:HALO + r0 + R, :]
            for w in range(1, WIN):
                s0 = HALO + r0 - DIL * w
                acc = acc + es[w] * vbuf[c, s0:s0 + R, :]
            obuf[r0:r0 + R, c * LANES:(c + 1) * LANES] = (acc * inv).astype(jnp.bfloat16)

    a = jnp.dot(obuf[...], wo_p[...], preferred_element_type=jnp.float32)
    g = jnp.dot(xn, wg[...], preferred_element_type=jnp.float32)
    u = jnp.dot(xn, wu[...], preferred_element_type=jnp.float32)
    h = (_gelu_tanh(g) * u).astype(jnp.bfloat16)
    b = jnp.dot(h, wd[...], preferred_element_type=jnp.float32)
    out_ref[...] = (x + a + b).astype(out_ref.dtype)


def _build(S, D, DF, T, R):
    NC = D // LANES
    kern = functools.partial(_kernel, T=T, R=R, D=D)
    any_spec = pl.BlockSpec(memory_space=pl.ANY)
    return pl.pallas_call(
        kern,
        grid=(S // T,),
        in_specs=[pl.BlockSpec((T, D), lambda i: (i, 0)),
                  any_spec, any_spec, any_spec, any_spec, any_spec],
        out_specs=pl.BlockSpec((T, D), lambda i: (i, 0)),
        out_shape=jax.ShapeDtypeStruct((S, D), jnp.bfloat16),
        scratch_shapes=[
            pltpu.VMEM((D, 3 * D), jnp.bfloat16),
            pltpu.VMEM((D, D), jnp.bfloat16),
            pltpu.VMEM((D, 3 * D), jnp.bfloat16),
            pltpu.VMEM((D, D), jnp.bfloat16),
            pltpu.VMEM((D, DF), jnp.bfloat16),
            pltpu.VMEM((D, DF), jnp.bfloat16),
            pltpu.VMEM((DF, D), jnp.bfloat16),
            pltpu.VMEM((NC, T, LANES), jnp.float32),
            pltpu.VMEM((NC, T + HALO, LANES), jnp.float32),
            pltpu.VMEM((NC, T + HALO, LANES), jnp.float32),
            pltpu.VMEM((T, D), jnp.bfloat16),
            pltpu.SemaphoreType.DMA((5,)),
        ],
        compiler_params=pltpu.CompilerParams(
            dimension_semantics=("arbitrary",),
            vmem_limit_bytes=100 * 1024 * 1024,
        ),
    )


@jax.jit
def pallas_parallel_sum__sliding_local_dilated__glu_gated_geglu__prompt_kernel(
    A_x: jax.Array,
    A_wqkv: jax.Array,
    A_wo: jax.Array,
    B_x: jax.Array,
    B_w_gate: jax.Array,
    B_w_up: jax.Array,
    B_w_down: jax.Array,
):
    B, S, D = A_x.shape
    DF = B_w_gate.shape[1]
    assert B == 1
    T, R = 256, 16
    out = _build(S, D, DF, T, R)(
        A_x.reshape(S, D), A_wqkv, A_wo, B_w_gate, B_w_up, B_w_down)
    return out.reshape(B, S, D)
```

```python
import functools

import jax
import jax.numpy as jnp
import jax.experimental.pallas as pl
import jax.experimental.pallas.tpu as pltpu

H = 32
DH = 16
WIN = 8
DIL = 2
HALO = 16
LANES = 128
EPS = 1e-5
NEG = -1e9
NT = (((1,), (1,)), ((), ()))


def _gelu_tanh(x):
    c = 0.7978845608028654
    return 0.5 * x * (1.0 + jnp.tanh(c * (x + 0.044715 * (x * x * x))))


def _kernel(x_hbm, wqkv_hbm, wo_hbm, wg_hbm, wu_hbm, wd_hbm, out_ref,
            xbuf, wqkv_raw, wo_raw, wtmp, wqkv_pt, wo_p, wg, wu, wd,
            xnbuf, qbuf, kbuf, vbuf, obuf, sems, *, S, T, R, D, DF, CH):
    i = pl.program_id(0)
    n = pl.num_programs(0)
    NC = D // LANES
    NJ = pl.cdiv(DF, LANES)
    never = i < 0
    f32 = jnp.float32
    bf16 = jnp.bfloat16

    cb = list(range(0, DF, CH)) + [DF]
    nch = len(cb) - 1

    def xtile(t):
        return xbuf[pl.ds(pl.multiple_of(t * T, T), T), :]

    def ln(t):
        x = xtile(t).astype(f32)
        mu = jnp.mean(x, axis=-1, keepdims=True)
        xc = x - mu
        var = jnp.mean(xc * xc, axis=-1, keepdims=True)
        xnbuf[...] = (xc * jax.lax.rsqrt(var + EPS)).astype(bf16)

    def halo(first):
        if first:
            kbuf[:, 0:HALO, :] = jnp.zeros((NC, HALO, LANES), f32)
            vbuf[:, 0:HALO, :] = jnp.zeros((NC, HALO, LANES), f32)
        else:
            kbuf[:, 0:HALO, :] = kbuf[:, T:T + HALO, :]
            vbuf[:, 0:HALO, :] = vbuf[:, T:T + HALO, :]

    def proj(p):
        y = jax.lax.dot_general(xnbuf[...], wqkv_pt[p * D:(p + 1) * D, :], NT,
                                preferred_element_type=f32)
        for c in range(NC):
            yc = y[:, c * LANES:(c + 1) * LANES]
            if p == 0:
                qbuf[c] = yc
            elif p == 1:
                kbuf[c, HALO:HALO + T, :] = yc
            else:
                vbuf[c, HALO:HALO + T, :] = yc

    def qkv_stage():
        halo(False)
        for p in range(3):
            proj(p)

    def attn_chunk(r0, gate, first):
        qc = [qbuf[c, r0:r0 + R, :] for c in range(NC)]
        if gate is not None:
            qc = [jnp.where(never, gate, q) for q in qc]
        ls = []
        for w in range(WIN):
            s0 = HALO + r0 - DIL * w
            p = qc[0] * kbuf[0, s0:s0 + R, :]
            for c in range(1, NC):
                p = p + qc[c] * kbuf[c, s0:s0 + R, :]
            p = p + pltpu.roll(p, 64, 1)
            p = p + pltpu.roll(p, 32, 1)
            if first and r0 < HALO and w > 0:
                pos = r0 + jax.lax.broadcasted_iota(jnp.int32, (R, LANES), 0)
                p = jnp.where(pos >= DIL * w, p, NEG)
            ls.append(p)
        m01 = jnp.maximum(ls[0], ls[1]); m23 = jnp.maximum(ls[2], ls[3])
        m45 = jnp.maximum(ls[4], ls[5]); m67 = jnp.maximum(ls[6], ls[7])
        m = jnp.maximum(jnp.maximum(m01, m23), jnp.maximum(m45, m67))
        es = [jnp.exp(l - m) for l in ls]
        den = ((es[0] + es[1]) + (es[2] + es[3])) + ((es[4] + es[5]) + (es[6] + es[7]))
        inv = 1.0 / den
        for c in range(NC):
            acc = es[0] * vbuf[c, HALO + r0:HALO + r0 + R, :]
            for w in range(1, WIN):
                s0 = HALO + r0 - DIL * w
                acc = acc + es[w] * vbuf[c, s0:s0 + R, :]
            obuf[r0:r0 + R, c * LANES:(c + 1) * LANES] = (acc * inv).astype(bf16)

    def attention(gates, first):
        nchunks = T // R
        for ci in range(nchunks):
            attn_chunk(ci * R, gates[ci * len(gates) // nchunks], first)

    def tiles(xn, w_ref, waits=None):
        out = []
        for j in range(NJ):
            lo, hi = j * LANES, min((j + 1) * LANES, DF)
            if waits is not None and lo in cb:
                waits[cb.index(lo)].wait()
            out.append(jax.lax.dot_general(xn, w_ref[lo:hi, :], NT, preferred_element_type=f32))
        return out

    def finish(bs):
        a = jnp.dot(obuf[...], wo_p[...], preferred_element_type=f32)
        b = jnp.concatenate(bs, axis=1)
        out_ref[...] = (xtile(i).astype(f32) + b + a).astype(out_ref.dtype)

    def down(h):
        return [jnp.dot(h, wd[:, c * LANES:(c + 1) * LANES], preferred_element_type=f32)
                for c in range(NC)]

    def perm_qkv(p):
        t = wqkv_raw[p].astype(f32).T
        if p == 0:
            t = t * (DH ** -0.5)
        for c in range(NC):
            wtmp[c, p * D:(p + 1) * D, :] = t[:, c * LANES:(c + 1) * LANES]
        for d in range(DH):
            for c in range(NC):
                wqkv_pt[p * D + d * H:p * D + (d + 1) * H, c * LANES:(c + 1) * LANES] = (
                    wtmp[c, pl.ds(p * D + d, H, stride=DH), :].astype(bf16))

    def perm_wo():
        wof = wo_raw[...].astype(f32)
        for c in range(NC):
            wtmp[c, 0:D, :] = wof[:, c * LANES:(c + 1) * LANES]
        for d in range(DH):
            for c in range(NC):
                wo_p[d * H:(d + 1) * H, c * LANES:(c + 1) * LANES] = (
                    wtmp[c, pl.ds(d, H, stride=DH), :].astype(bf16))

    @pl.when(i == 0)
    def _():
        cp_qkv = [pltpu.make_async_copy(wqkv_hbm.at[:, p * D:(p + 1) * D], wqkv_raw.at[p],
                                        sems.at[p]) for p in range(3)]
        cp_g = pltpu.make_async_copy(wg_hbm, wg, sems.at[3])
        cp_u = pltpu.make_async_copy(wu_hbm, wu, sems.at[4])
        cp_d = pltpu.make_async_copy(wd_hbm, wd, sems.at[5])
        cp_wo = pltpu.make_async_copy(wo_hbm, wo_raw, sems.at[6])
        cp_x0 = pltpu.make_async_copy(x_hbm.at[0:T, :], xbuf.at[0:T, :], sems.at[7])
        cp_x1 = pltpu.make_async_copy(x_hbm.at[T:2 * T, :], xbuf.at[T:2 * T, :], sems.at[9])
        cp_xr = pltpu.make_async_copy(x_hbm.at[2 * T:S, :], xbuf.at[2 * T:S, :], sems.at[8])
        for cp in [cp_qkv[0], cp_x0, cp_qkv[1], cp_qkv[2], cp_g, cp_u, cp_d, cp_wo, cp_x1, cp_xr]:
            cp.start()

        cp_x0.wait()
        ln(0)
        halo(True)
        cp_qkv[0].wait()
        perm_qkv(0)
        cp_qkv[1].wait()
        perm_qkv(1)
        proj(0)
        cp_qkv[2].wait()
        perm_qkv(2)
        proj(1)
        cp_g.wait()
        proj(2)
        xn = xnbuf[...]
        gs = tiles(xn, wg)
        attention([g[0:R, :] for g in gs[:NJ - 1]], True)
        cp_u.wait()
        us = tiles(xn, wu)
        h = jnp.concatenate([(_gelu_tanh(g) * u).astype(bf16) for g, u in zip(gs, us)], axis=1)
        cp_d.wait()
        cp_wo.wait()
        cp_x1.wait()
        perm_wo()
        finish(down(h))
        ln(i + 1)
        qkv_stage()
        cp_xr.wait()

    def main_stage():
        xn = xnbuf[...]
        gs = tiles(xn, wg)
        attention([g[0:R, :] for g in gs[:NJ - 1]], False)
        us = tiles(xn, wu)
        h = jnp.concatenate([(_gelu_tanh(g) * u).astype(bf16) for g, u in zip(gs, us)], axis=1)
        finish(down(h))

    @pl.when(jnp.logical_and(i > 0, i < n - 1))
    def _():
        main_stage()
        ln(i + 1)
        qkv_stage()

    @pl.when(i == n - 1)
    def _():
        main_stage()


def _build(S, D, DF, T, R, CH):
    NC = D // LANES
    n = S // T
    nch = pl.cdiv(DF, CH)
    kern = functools.partial(_kernel, S=S, T=T, R=R, D=D, DF=DF, CH=CH)
    any_spec = pl.BlockSpec(memory_space=pl.ANY)
    return pl.pallas_call(
        kern,
        grid=(n,),
        in_specs=[any_spec,
                  any_spec, any_spec, any_spec, any_spec, any_spec],
        out_specs=pl.BlockSpec((T, D), lambda i: (i, 0)),
        out_shape=jax.ShapeDtypeStruct((S, D), jnp.bfloat16),
        scratch_shapes=[
            pltpu.VMEM((S, D), jnp.bfloat16),
            pltpu.VMEM((3, D, D), jnp.bfloat16),
            pltpu.VMEM((D, D), jnp.bfloat16),
            pltpu.VMEM((NC, 3 * D, LANES), jnp.float32),
            pltpu.VMEM((3 * D, D), jnp.bfloat16),
            pltpu.VMEM((D, D), jnp.bfloat16),
            pltpu.VMEM((DF, D), jnp.bfloat16),
            pltpu.VMEM((DF, D), jnp.bfloat16),
            pltpu.VMEM((DF, D), jnp.bfloat16),
            pltpu.VMEM((T, D), jnp.bfloat16),
            pltpu.VMEM((NC, T, LANES), jnp.float32),
            pltpu.VMEM((NC, T + HALO, LANES), jnp.float32),
            pltpu.VMEM((NC, T + HALO, LANES), jnp.float32),
            pltpu.VMEM((T, D), jnp.bfloat16),
            pltpu.SemaphoreType.DMA((10,)),
        ],
        compiler_params=pltpu.CompilerParams(
            dimension_semantics=("arbitrary",),
            vmem_limit_bytes=100 * 1024 * 1024,
        ),
    )

CFG = dict(T=256, R=16, CH=384)

@jax.jit
def pallas_parallel_sum__sliding_local_dilated__glu_gated_geglu__prompt_kernel(
    A_x, A_wqkv, A_wo, B_x, B_w_gate, B_w_up, B_w_down):
    B, S, D = A_x.shape
    DF = B_w_gate.shape[1]
    x2 = A_x.reshape(S, D)
    out = _build(S, D, DF, **CFG)(
        x2, A_wqkv, A_wo, B_w_gate.T, B_w_up.T, B_w_down)
    return out.reshape(B, S, D)
```

```python
import functools

import jax
import jax.numpy as jnp
import jax.experimental.pallas as pl
import jax.experimental.pallas.tpu as pltpu

H = 32
DH = 16
WIN = 8
DIL = 2
HALO = 16
LANES = 128
EPS = 1e-5
NEG = -1e9
NT = (((1,), (1,)), ((), ()))


def _gelu_tanh(x):
    c = 0.7978845608028654
    return 0.5 * x * (1.0 + jnp.tanh(c * (x + 0.044715 * (x * x * x))))


def _kernel(x_hbm, wqkv_hbm, wo_hbm, wg_hbm, wu_hbm, wd_hbm, out_ref,
            xbuf, wqkv_raw, wo_raw, wtmp, wqkv_pt, wo_p, wg, wu, wd,
            xnbuf, qbuf, kbuf, vbuf, obuf, sems, *, S, T, R, D, DF):
    i = pl.program_id(0)
    n = pl.num_programs(0)
    NC = D // LANES
    NJ = pl.cdiv(DF, LANES)
    never = i < 0
    f32 = jnp.float32
    bf16 = jnp.bfloat16

    def xtile(t):
        return xbuf[pl.ds(pl.multiple_of(t * T, T), T), :]

    def ln(t, off=0):
        x = xtile(t).astype(f32)
        mu = jnp.mean(x, axis=-1, keepdims=True)
        xc = x - mu
        var = jnp.mean(xc * xc, axis=-1, keepdims=True)
        xnbuf[off:off + T, :] = (xc * jax.lax.rsqrt(var + EPS)).astype(bf16)

    def halo(first):
        if first:
            kbuf[:, 0:HALO, :] = jnp.zeros((NC, HALO, LANES), f32)
            vbuf[:, 0:HALO, :] = jnp.zeros((NC, HALO, LANES), f32)
        else:
            kbuf[:, 0:HALO, :] = kbuf[:, T:T + HALO, :]
            vbuf[:, 0:HALO, :] = vbuf[:, T:T + HALO, :]

    def proj(p, M=T):
        y = jax.lax.dot_general(xnbuf[0:M, :], wqkv_pt[p * D:(p + 1) * D, :], NT,
                                preferred_element_type=f32)
        for c in range(NC):
            yc = y[:, c * LANES:(c + 1) * LANES]
            if p == 0:
                qbuf[c, 0:M, :] = yc
            elif p == 1:
                kbuf[c, HALO:HALO + M, :] = yc
            else:
                vbuf[c, HALO:HALO + M, :] = yc

    def qkv_stage():
        halo(False)
        for p in range(3):
            proj(p)

    def attn_chunk(r0, gate, first):
        qc = [jnp.where(never, gate, qbuf[c, r0:r0 + R, :]) for c in range(NC)]
        ls = []
        for w in range(WIN):
            s0 = HALO + r0 - DIL * w
            p = qc[0] * kbuf[0, s0:s0 + R, :]
            for c in range(1, NC):
                p = p + qc[c] * kbuf[c, s0:s0 + R, :]
            p = p + pltpu.roll(p, 64, 1)
            p = p + pltpu.roll(p, 32, 1)
            if first and r0 < HALO and w > 0:
                pos = r0 + jax.lax.broadcasted_iota(jnp.int32, (R, LANES), 0)
                p = jnp.where(pos >= DIL * w, p, NEG)
            ls.append(p)
        m = jnp.maximum(jnp.maximum(jnp.maximum(ls[0], ls[1]), jnp.maximum(ls[2], ls[3])),
                        jnp.maximum(jnp.maximum(ls[4], ls[5]), jnp.maximum(ls[6], ls[7])))
        es = [jnp.exp(l - m) for l in ls]
        den = ((es[0] + es[1]) + (es[2] + es[3])) + ((es[4] + es[5]) + (es[6] + es[7]))
        inv = 1.0 / den
        for c in range(NC):
            acc = es[0] * vbuf[c, HALO + r0:HALO + r0 + R, :]
            for w in range(1, WIN):
                s0 = HALO + r0 - DIL * w
                acc = acc + es[w] * vbuf[c, s0:s0 + R, :]
            obuf[r0:r0 + R, c * LANES:(c + 1) * LANES] = (acc * inv).astype(bf16)

    def attention(gates, first):
        nchunks = T // R
        for ci in range(nchunks):
            attn_chunk(ci * R, gates[ci * len(gates) // nchunks][0:R, :], first)

    def tiles(xn, w_ref):
        return [jax.lax.dot_general(xn, w_ref[j * LANES:min((j + 1) * LANES, DF), :], NT,
                                    preferred_element_type=f32) for j in range(NJ)]

    def geglu(gs, us):
        return jnp.concatenate([(_gelu_tanh(g) * u).astype(bf16) for g, u in zip(gs, us)],
                               axis=1)

    def finish(h):
        b = jnp.concatenate(
            [jnp.dot(h, wd[:, c * LANES:(c + 1) * LANES], preferred_element_type=f32)
             for c in range(NC)], axis=1)
        a = jnp.dot(obuf[...], wo_p[...], preferred_element_type=f32)
        out_ref[...] = (xtile(i).astype(f32) + b + a).astype(out_ref.dtype)

    def perm_qkv(p):
        t = wqkv_raw[p].astype(f32).T
        if p == 0:
            t = t * (DH ** -0.5)
        for c in range(NC):
            wtmp[c, p * D:(p + 1) * D, :] = t[:, c * LANES:(c + 1) * LANES]
        for d in range(DH):
            for c in range(NC):
                wqkv_pt[p * D + d * H:p * D + (d + 1) * H, c * LANES:(c + 1) * LANES] = (
                    wtmp[c, pl.ds(p * D + d, H, stride=DH), :].astype(bf16))

    def perm_wo():
        wof = wo_raw[...].astype(f32)
        for c in range(NC):
            wtmp[c, 0:D, :] = wof[:, c * LANES:(c + 1) * LANES]
        for d in range(DH):
            for c in range(NC):
                wo_p[d * H:(d + 1) * H, c * LANES:(c + 1) * LANES] = (
                    wtmp[c, pl.ds(d, H, stride=DH), :].astype(bf16))

    @pl.when(i == 0)
    def _():
        cp_qkv = [pltpu.make_async_copy(wqkv_hbm.at[:, p * D:(p + 1) * D], wqkv_raw.at[p],
                                        sems.at[p]) for p in range(3)]
        cp_g = pltpu.make_async_copy(wg_hbm, wg, sems.at[3])
        cp_u = pltpu.make_async_copy(wu_hbm, wu, sems.at[4])
        cp_d = pltpu.make_async_copy(wd_hbm, wd, sems.at[5])
        cp_wo = pltpu.make_async_copy(wo_hbm, wo_raw, sems.at[6])
        cp_x0 = pltpu.make_async_copy(x_hbm.at[0:2 * T, :], xbuf.at[0:2 * T, :], sems.at[7])
        cp_xr = pltpu.make_async_copy(x_hbm.at[2 * T:S, :], xbuf.at[2 * T:S, :], sems.at[8])
        for cp in [cp_x0, cp_qkv[0], cp_qkv[1], cp_qkv[2], cp_g, cp_u, cp_d, cp_wo, cp_xr]:
            cp.start()

        halo(True)
        wtmp[:, 3 * D:3 * D + DH, :] = jnp.zeros((NC, DH, LANES), f32)
        cp_x0.wait()
        ln(0)
        ln(1, T)
        cp_qkv[0].wait()
        perm_qkv(0)
        cp_qkv[1].wait()
        perm_qkv(1)
        proj(0, 2 * T)
        proj(1, 2 * T)
        cp_qkv[2].wait()
        cp_g.wait()
        xn = xnbuf[0:T, :]
        perm_qkv(2)
        gs = tiles(xn, wg)
        proj(2, 2 * T)
        cp_u.wait()
        cp_d.wait()
        cp_wo.wait()
        us = tiles(xn, wu)
        attention(us[:NJ - 1], True)
        h = geglu(gs, us)
        perm_wo()
        finish(h)
        xnbuf[0:T, :] = xnbuf[T:2 * T, :]
        qbuf[:, 0:T, :] = qbuf[:, T:2 * T, :]
        kbuf[:, 0:HALO + T, :] = kbuf[:, T:HALO + 2 * T, :]
        vbuf[:, 0:HALO + T, :] = vbuf[:, T:HALO + 2 * T, :]
        cp_xr.wait()

    def main_stage():
        xn = xnbuf[0:T, :]
        gs = tiles(xn, wg)
        attention(gs[:NJ - 1], False)
        us = tiles(xn, wu)
        finish(geglu(gs, us))

    @pl.when(jnp.logical_and(i > 0, i < n - 1))
    def _():
        main_stage()
        ln(i + 1)
        qkv_stage()

    @pl.when(i == n - 1)
    def _():
        main_stage()


def _build(S, D, DF, T, R):
    NC = D // LANES
    n = S // T
    assert S % T == 0 and n >= 3 and T % R == 0 and D == H * DH and D % LANES == 0
    kern = functools.partial(_kernel, S=S, T=T, R=R, D=D, DF=DF)
    any_spec = pl.BlockSpec(memory_space=pl.ANY)
    return pl.pallas_call(
        kern,
        grid=(n,),
        in_specs=[any_spec] * 6,
        out_specs=pl.BlockSpec((T, D), lambda i: (i, 0)),
        out_shape=jax.ShapeDtypeStruct((S, D), jnp.bfloat16),
        scratch_shapes=[
            pltpu.VMEM((S, D), jnp.bfloat16),
            pltpu.VMEM((3, D, D), jnp.bfloat16),
            pltpu.VMEM((D, D), jnp.bfloat16),
            pltpu.VMEM((NC, 3 * D + DH, LANES), jnp.float32),
            pltpu.VMEM((3 * D, D), jnp.bfloat16),
            pltpu.VMEM((D, D), jnp.bfloat16),
            pltpu.VMEM((DF, D), jnp.bfloat16),
            pltpu.VMEM((DF, D), jnp.bfloat16),
            pltpu.VMEM((DF, D), jnp.bfloat16),
            pltpu.VMEM((2 * T, D), jnp.bfloat16),
            pltpu.VMEM((NC, 2 * T, LANES), jnp.float32),
            pltpu.VMEM((NC, 2 * T + HALO, LANES), jnp.float32),
            pltpu.VMEM((NC, 2 * T + HALO, LANES), jnp.float32),
            pltpu.VMEM((T, D), jnp.bfloat16),
            pltpu.SemaphoreType.DMA((9,)),
        ],
        compiler_params=pltpu.CompilerParams(
            dimension_semantics=("arbitrary",),
            vmem_limit_bytes=100 * 1024 * 1024,
        ),
    )


@jax.jit
def pallas_parallel_sum__sliding_local_dilated__glu_gated_geglu__prompt_kernel(
    A_x: jax.Array,
    A_wqkv: jax.Array,
    A_wo: jax.Array,
    B_x: jax.Array,
    B_w_gate: jax.Array,
    B_w_up: jax.Array,
    B_w_down: jax.Array,
):
    B, S, D = A_x.shape
    DF = B_w_gate.shape[1]
    assert B == 1
    out = _build(S, D, DF, T=256, R=16)(
        A_x.reshape(S, D), A_wqkv, A_wo, B_w_gate.T, B_w_up.T, B_w_down)
    return out.reshape(B, S, D)
```
